```python
import os as _os
_os.environ.setdefault("JAX_PLATFORMS", "cpu")
import jax
import jax.numpy as jnp

def _softmax(x, axis=-1):
    return jax.nn.softmax(x, axis=axis)
def _gelu(x):
    return jax.nn.gelu(x, approximate=True)
def _silu(x):
    return jax.nn.silu(x)
def _sigmoid(x):
    return jax.nn.sigmoid(x)
def _layernorm(x, axis=-1, eps=1e-5):
    m = jnp.mean(x, axis=axis, keepdims=True)
    v = jnp.var(x, axis=axis, keepdims=True)
    return (x - m) / jnp.sqrt(v + eps)
def _scatter_add(tgt, idx, src, axis=0):
    return tgt.at[idx].add(src)
def _segment_sum(src, seg, n):
    return jax.ops.segment_sum(src, seg, n)
class _Rng:
    def __init__(self, key):
        self._k = key
    def _next(self):
        self._k, sub = jax.random.split(self._k)
        return sub
    def normal(self, shape):
        return jax.random.normal(self._next(), shape, dtype=jnp.bfloat16)
    def randint(self, lo, hi, shape):
        return jax.random.randint(self._next(), shape, lo, hi, dtype=jnp.int32)
    def uniform(self, shape, lo=0.0, hi=1.0):
        return jax.random.uniform(self._next(), shape, jnp.bfloat16, lo, hi)
    def permutation(self, n):
        return jax.random.permutation(self._next(), n)


kernel_name = 'gated_mix__linear_attn_block__swiglu_ffn__prompt'

def setup_inputs():
    _rng = _Rng(jax.random.key(int.from_bytes(__import__("os").urandom(4), "little")))
    _w = (lambda a: (lambda t: t.astype(jnp.bfloat16) if jnp.issubdtype(t.dtype, jnp.floating) else t)(jnp.asarray(a)))
    def _A_setup():
        B, S, D = 1, 2048, 512
        return {
            "x": _w((lambda *s: _rng.normal(s) * 0.05)(B, S, D)),
            "wqkv": _w((lambda *s: _rng.normal(s) * 0.8)(D, 3 * D)),
            "wo": _w((lambda *s: _rng.normal(s) * 0.05)(D, D)),
        }
    _A_in = _A_setup()

    def _B_setup():
        B, S, D, F = 1, 2048, 512, 1792
        return {
            "x": _w((lambda *s: _rng.normal(s) * 0.05)(B, S, D)),
            "w_gate": _w((lambda *s: _rng.normal(s) * 0.1)(D, F)),
            "w_up": _w((lambda *s: _rng.normal(s) * 0.1)(D, F)),
            "w_down": _w((lambda *s: _rng.normal(s) * 0.1)(F, D)),
        }
    _B_in = _B_setup()

    return {
        "A_x": _A_in["x"],
        "A_wqkv": _A_in["wqkv"],
        "A_wo": _A_in["wo"],
        "B_x": _B_in["x"],
        "B_w_gate": _B_in["w_gate"],
        "B_w_up": _B_in["w_up"],
        "B_w_down": _B_in["w_down"],
        "gate_w": _w((lambda *s: _rng.normal(s) * 0.05)(512) * 16.0),
    }

def reference(A_x, A_wqkv, A_wo, B_x, B_w_gate, B_w_up, B_w_down, gate_w):
    def _A_ref(x, wqkv, wo):
        B, S, D = x.shape
        H = 32; Dh = D // H
        qkv = (lambda x, *d: x.transpose(*d))((x @ wqkv).reshape(B, S, 3, H, Dh), 2, 0, 3, 1, 4)
        q, k, v = qkv[0], qkv[1], qkv[2]
        phi = lambda t: jnp.where(t > 0, t + 1, jnp.exp(t)) + 1e-6
        pq, pk = phi(q), phi(k)
        kv = jnp.einsum("bhsd,bhse->bhde", pk, v)
        z = jnp.einsum("bhsd->bhd", pk)
        num = jnp.einsum("bhqd,bhde->bhqe", pq, kv)
        den = jnp.einsum("bhqd,bhd->bhq", pq, z)[..., None] + 1e-6
        o = num / den
        return (lambda x, *d: x.transpose(*d))(o, 0, 2, 1, 3).reshape(B, S, D) @ wo

    def _B_ref(x, w_gate, w_up, w_down):
        g = _silu(x @ w_gate)
        u = x @ w_up
        return (g * u) @ w_down

    x = A_x
    g = _sigmoid((x * gate_w).sum(-1, keepdims=True))
    a = _A_ref(x, A_wqkv, A_wo)
    b = _B_ref(x, B_w_gate, B_w_up, B_w_down)
    return g * a + (1 - g) * b
```

```python
import jax, jax.numpy as jnp
from jax import lax
import jax.experimental.pallas as pl
import jax.experimental.pallas.tpu as pltpu

S, D, F, H, DH = 2048, 512, 1792, 32, 16
T = 128
C = 16
NB = 4
NC = T // C
PITCH = 17
f32, bf16, u32 = jnp.float32, jnp.bfloat16, jnp.uint32

LHS = [((0,0,1),(1,1,1)), ((1,0,1),(1,1,1)), ((0,0,1),), ((1,1,1),), ((0,0,1),(0,1,1)), ((1,0,1),(0,0,-1)), ((0,1,1),(1,1,-1))]
L2R = [0, 2, 6, 5, 3, 4, 1]
RHS = [LHS[i] for i in L2R]
OUT = [((0,0,1),(1,1,1)), ((1,0,1),(1,1,-1)), ((0,1,1),(1,1,1)), ((0,0,1),(1,0,1)), ((0,1,1),(0,0,-1)), ((1,1,1),), ((0,0,1),)]
ORDER = (0, 5, 6, 1, 2, 3, 4)
OORDER = (2, 3, 4, 1, 0, 6, 5)
QUAD = ((0, 0), (0, 1), (1, 0), (1, 1))

def comb(terms, blk):
    acc = None
    for i, j, s in terms:
        v = blk(i, j)
        acc = v if acc is None else (acc + v if s > 0 else acc - v)
    return acc
def out4(m):
    return {(0,0): (m[0] + m[6]) + (m[3] - m[4]), (0,1): m[2] + m[4], (1,0): m[1] + m[3], (1,1): (m[0] + m[5]) + (m[2] - m[1])}
def dot(a, b):
    return jnp.dot(a, b, preferred_element_type=f32)
def dot_nt(a, b):
    return lax.dot_general(a, b, (((1,), (1,)), ((), ())), preferred_element_type=f32)
def phi(t):
    return jnp.where(t > 0, t + 1.0, jnp.exp(t)) + 1e-6
def ts(i):
    return slice(i * T, (i + 1) * T)
def cat(vs, ax):
    return jnp.concatenate(vs, axis=ax) if len(vs) > 1 else vs[0]
def merge(*lists):
    keyed = [((k + 0.5) / len(l), j, k) for j, l in enumerate(lists) for k in range(len(l))]
    return [lists[j][k] for _, j, k in sorted(keyed)]
def part(l, i, n):
    return l[len(l) * i // n: len(l) * (i + 1) // n]
def ds(start, n, align):
    return pl.ds(start if isinstance(start, int) else pl.multiple_of(start, align), n)

class Buf:
    def __init__(self, ref, zero):
        self.ref, self.zero = ref, zero
    def st(self, slot, tile, c, v, col=0):
        self.ref[slot, ds(C + tile * T + c * C, v.shape[0], C), ts(col)] = v.astype(self.ref.dtype)
    def ld(self, slot, tile, c=0, n=C, col=0):
        return self.ref[slot, ds(C + tile * T + c * C, n, C), ts(col)].astype(f32)
    def words(self, slot, tile, a, n):
        return self.ref.bitcast(u32)[slot, pl.ds((C + tile * T + a * C) // 2, n // 2), :]
    def mx(self, slot, tile, n=T):
        return pltpu.bitcast(self.words(slot, tile, 0, n), bf16)
    def token(self):
        r = self.ref if self.ref.dtype == f32 else self.ref.bitcast(u32)
        v = r[0, ds(self.zero * 8, 8, 8), 0:T]
        return pltpu.bitcast(v, u32) if v.dtype == f32 else v
    def release(self, v):
        n = 8 if self.ref.dtype == f32 else C
        self.ref[0, ds(self.zero * n, n, n), 0:T] = v[0:n].astype(self.ref.dtype)

def make(lead=1, lag=10, xlag=16, U1=1, U2=1, U3=1, flags=None, only=None):
    def kernel(x_h, wqkv_h, wo_h, wg_h, wu_h, wd_h, gw_h, o_h, wv_v, wo_v, gw_v, *rest):
        *refs, sems, osem, zsem = rest
        zero = pl.semaphore_read(zsem)
        never = zero != 0
        bufs = [Buf(r, zero) for r in refs]
        (xr, wqr, wkr, wgr, wur, wdr, ob, pb, gb, zb, zr, wb, xc, w1c, wkc, wqc, pkc, w2c, hc, hs, ks, tk, tq, tw), rings = bufs[:-3], bufs[-3:]

        def rows(buf, n, slot=0):
            return buf.ref.at[slot, pl.ds(C, n)]
        cp = {}
        def fetch(name, src, dst):
            cp[name] = pltpu.make_async_copy(src, dst, sems.at[len(cp)])
            cp[name].start()
        def fetch_x(b):
            fetch(('x', b), x_h.at[pl.ds(b * 4 * T, 4 * T)], rows(xr, 4 * T, b))
        def fetch_w1(g):
            fetch(('wg', g), wg_h.at[:, pl.ds(g * 2 * T, 2 * T)], rows(wgr, D, g))
            fetch(('wu', g), wu_h.at[:, pl.ds(g * 2 * T, 2 * T)], rows(wur, D, g))
        def wait(*names):
            for n in names: cp[n].wait()
        fetch_x(0); fetch_w1(0); fetch('gw', gw_h, gw_v); fetch_x(1); fetch_w1(1); fetch_x(2); fetch_x(3)
        fetch('wk', wqkv_h.at[:, pl.ds(D, D)], rows(wkr, D))
        for g in range(2, 7): fetch_w1(g)
        fetch('wq', wqkv_h.at[:, pl.ds(0, D)], rows(wqr, D))
        fetch('wv', wqkv_h.at[:, pl.ds(2 * D, D)], wv_v)
        fetch('wo', wo_h, wo_v)
        fetch('wd', wd_h, rows(wdr, F))
        for bf in bufs: bf.release(jnp.zeros((C, T), f32))

        def operands(table, cell, store, gates, out, cost, chunks=range(NC), outer=range(7)):
            def task(r1, c):
                o = {q: comb(table[r1], lambda i1, j1: cell(2 * i1 + q[0], 2 * j1 + q[1], c)) for q in QUAD}
                for r2 in range(7):
                    store(r1 * 7 + r2, c, comb(table[r2], lambda i, j: o[i, j]))
            return [(cost, gates, lambda r1=r1, c=c: task(r1, c), [out], lag) for r1 in outer for c in chunks]
        def x_ops(b):
            return operands(LHS, lambda i, j, c: xr.ld(b, i, c, col=j), lambda r, c, v: xc.st(b, r, c, v), [xr], xc, 37)
        def gate(b):
            def task(i, c):
                gw = 0.5 * gw_v[...].astype(f32).reshape(1, D)
                p = [xr.ld(b, i, c, col=j) * gw[:, ts(j)] for j in range(4)]
                t = 0.5 * jnp.tanh(jnp.sum((p[0] + p[1]) + (p[2] + p[3]), axis=1, keepdims=True))
                gb.st(b, i, c, jnp.broadcast_to(0.5 - t, (C, T)))
            return [(30, [xr], lambda i=i, c=c: task(i, c), [gb], xlag) for c in range(NC) for i in range(4)]
        def w1_ops(g, chunks=range(NC)):
            cell = lambda k, n, c: (wgr, wgr, wur, wur)[n].ld(g, k, c, col=(0, 1, 1, 0)[n])
            return operands(RHS, cell, lambda r, c, v: w1c.st(g, r, c, v), [wgr, wur], w1c, 37, chunks)
        def st_heads(dst, slot, j, v):
            for h in range(T // DH):
                dst.ref[slot, pl.ds(C + (j * (T // DH) + h) * PITCH, DH), :] = v[h * DH:(h + 1) * DH]
        def permuted(src, slot, j, c, n=C):
            j0 = j * T + c * C
            return src.ref[slot, pl.ds(C + (j0 % H) * PITCH + j0 // H, n, stride=PITCH), :]
        def transpose(src, dst):
            task = lambda k, j: st_heads(dst, k, j, src.ld(0, k, 0, T, col=j).T)
            return [(40, [src], lambda k=k, j=j: task(k, j), [dst], xlag) for k in range(4) for j in range(4)]
        def wk_ops():
            cell = lambda k, j, c: tk.ref[k, pl.ds(C + (j * NC + c) * PITCH, C), :]
            return operands(RHS, cell, lambda r, c, v: wkc.st(0, r, c, v), [tk], wkc, 23)
        def wq_ops():
            return operands(RHS, lambda k, j, c: permuted(tq, k, j, c), lambda r, c, v: wqc.st(0, r, c, v), [tq], wqc, 23)
        def w2_ops(s):
            cell = (lambda j, n, c: permuted(tw, n, j, c)) if s == 3 else (lambda k, n, c: wdr.ld(0, 4 * s + k, c, col=n))
            return operands(RHS, cell, lambda r, c, v: w2c.st(0, r * 4 + s, c, v), [tw if s == 3 else wdr], w2c, 23 if s == 3 else 37)
        def w2_tail():
            def task(n2, c):
                o = {(k, n1): wdr.ld(0, 12 + k, c, col=2 * n1 + n2) for k, n1 in QUAD}
                for r1 in range(7):
                    w2c.st(0, 196 + r1 * 2 + n2, c, comb(RHS[r1], lambda i, j: o[i, j]))
            return [(25, [wdr], lambda n2=n2, c=c: task(n2, c), [w2c], lag) for n2 in range(2) for c in range(NC)]
        def h_ops(b, r1):
            tasks = []
            for s in range(4):
                cell = (lambda i, k, c: hs.ld(b, i * 18 + 14 + k, c) * wb.ld(b, i, c)) if s == 3 else (lambda i, k, c, s=s: hs.ld(b, i * 18 + 4 * s + k, c))
                tasks += operands(LHS, cell, lambda r, c, v, s=s: hc.st(0, r * 4 + s, c, v), [hs], hc, 23, outer=[r1])
            def tail(c):
                for i2 in range(2):
                    hc.st(0, 196 + r1 * 2 + i2, c, comb(LHS[r1], lambda i1, k: hs.ld(b, (2 * i1 + i2) * 18 + 12 + k, c)))
            return tasks + [(6, [hs], lambda c=c: tail(c), [hc], lag) for c in range(NC)]
        def pk_ops(b):
            def zsum(c):
                for j in range(4):
                    p = [ks.ld(0, j * 4 + i, c) for i in range(4)]
                    zb.st(b, j, c, (p[0] + p[1]) + (p[2] + p[3]))
            return merge(operands(LHS, lambda j, i, c: ks.ld(0, j * 4 + i, c), lambda r, c, v: pkc.st(b, r, c, v), [ks], pkc, 23),
                         [(24, [ks], lambda c=c: zsum(c), [zb], lag) for c in range(NC)])
        def z_lanes():
            def task(j):
                p = [zb.ld(b, j, 0, T) for b in range(4)]
                st_heads(tk, 0, j, jnp.broadcast_to(jnp.sum((p[0] + p[1]) + (p[2] + p[3]), axis=1, keepdims=True), (T, T)))
            return [(60, [zb], lambda j=j: task(j), [tk], xlag) for j in range(4)]
        def z_rows():
            task = lambda j: zr.st(0, 0, j, cat([permuted(tk, 0, j, c) for c in range(NC)], 0).T[0:C])
            return [(30, [tk], lambda j=j: task(j), [zr], xlag) for j in range(4)]

        def finish(rb, fn, cost, outs, lg):
            def task(c, i2):
                o = [out4([rb.ld(0, r1 * 4 + i2 * 2 + j2, c) for r1 in range(7)]) for j2 in range(2)]
                for i1 in range(2):
                    fn(2 * i1 + i2, c, [o[j2][i1, j1] for j1, j2 in QUAD])
            return [(cost, [rb], lambda c=c, i2=i2: task(c, i2), outs, lg) for c in range(NC) for i2 in range(2)]
        def post_f(rb, b, g):
            def fn(i, c, v):
                gm = gb.ld(b, i, c)
                for k, (G, U) in enumerate(((v[0], v[3]), (v[1], v[2]))):
                    hg = 0.5 * G
                    hs.st(b, i * 18 + 2 * g + k, c, (hg * jnp.tanh(hg) + hg) * (U * gm))
            return finish(rb, fn, 80, [hs], lag)
        def post_k(rb):
            def fn(i, c, v):
                for j in range(4): ks.st(0, j * 4 + i, c, phi(v[j]))
            return finish(rb, fn, 112, [ks], lag)
        def post_q(rb, b):
            def fn(i, c, v):
                p = [phi(a) for a in v]
                for j in range(4): hs.st(b, i * 18 + 14 + j, c, p[j])
                t = [p[j] * zr.ld(0, 0, j) for j in range(4)]
                ks.st(0, i, c, (t[0] + t[1]) + (t[2] + t[3]))
            return finish(rb, fn, 140, [hs, ks], lag)
        def q_norm(b):
            def task(c):
                for i in range(4):
                    t = ks.ld(0, i, c)
                    t = t + pltpu.roll(t, 64, 1)
                    t = t + pltpu.roll(t, 32, 1)
                    wb.st(b, i, c, (1.0 - gb.ld(b, i, c)) / (t + 1e-6))
            return [(100, [ks], lambda c=c: task(c), [wb], xlag + 4) for c in range(NC)]

        clock = [0]
        due = {}
        def barrier():
            due.clear(); clock[0] = 0
        def spread(tasks, slots):
            total = sum(t[0] for t in tasks)
            pos = dict(spent=0, done=0, d=0)
            def emit():
                pos['d'] += 1; now = []
                while pos['done'] < len(tasks) and pos['spent'] * (slots - lead) < total * (pos['d'] - lead):
                    now.append(tasks[pos['done']]); pos['spent'] += now[-1][0]; pos['done'] += 1
                return now
            return emit
        def product(fn, lhs, rhs, emit):
            t0 = clock[0]; cols = []
            for a, (bf, slot, tile) in enumerate(lhs):
                toks = due.pop(t0 + a, None)
                if toks:
                    k = 2 * (a if len(lhs) > 1 else t0 % 4)
                    w = [bf.words(slot, tile, c, C) for c in range(NC)]; tok = toks[0]
                    for other in toks[1:]: tok = tok | other
                    w[k] = jnp.where(never, tok, w[k])
                    cols.append(pltpu.bitcast(cat(w, 0), bf16))
                else:
                    cols.append(bf.mx(slot, tile))
            m = fn(cat(cols, 1), rhs)
            for a in range(len(lhs)):
                k = 32 * (a if len(lhs) > 1 else t0 % 4)
                gated, outs = [], {}
                for _, gates, task, written, lg in emit():
                    for g in gates:
                        if g not in gated:
                            g.release(m[k:k + C]); gated.append(g)
                    task()
                    for o in written: outs[bufs.index(o)] = max(lg, outs.get(bufs.index(o), 0))
                for o, lg in outs.items(): due.setdefault(t0 + a + lg, []).append(bufs[o].token())
            clock[0] += len(lhs)
            return m
        def unit(rb, fn, lhs, rhs, side, tail=0):
            emit = spread(merge(*side), 49 - tail)
            for r1 in range(7):
                o = out4({r2: product(fn, [lhs(r1 * 7 + r2)], rhs(r1 * 7 + r2), emit) for r2 in ORDER})
                for i2, j2 in QUAD:
                    rb.st(0, r1 * 4 + i2 * 2 + j2, 0, o[i2, j2])
        def wide_unit(lhs, rhs, extra, emit_for, store):
            acc = {}
            left = {q: sum(t[:2] == q for o in OUT for t in o) for q in QUAD}
            for a, r1 in enumerate(OORDER):
                emit = emit_for(a)
                o = out4({r2: product(dot, lhs(r1 * 7 + r2), rhs(r1 * 7 + r2), emit) for r2 in ORDER})
                if extra:
                    o = {q: o[q] + product(dot, *extra(r1, *q), emit) for q in QUAD}
                for i1, j1, sg in OUT[r1]:
                    left[i1, j1] -= 1
                    for i2, j2 in QUAD:
                        key = (2 * i1 + i2, 2 * j1 + j2)
                        acc[key] = o[i2, j2] if key not in acc else (acc[key] + o[i2, j2] if sg > 0 else acc[key] - o[i2, j2])
                        if not left[i1, j1]: store(*key, acc[key])
        def run(tasks):
            for t in tasks: t[2]()
        def Fu(rb, b, g, *side, **kw):
            unit(rb, dot, lambda r: (xc, b, r), lambda r: w1c.mx(g, r), side, **kw)
            return post_f(rb, b, g)
        def Ku(rb, b, *side, **kw):
            unit(rb, dot_nt, lambda r: (wkc, 0, r), lambda r: xc.mx(b, r), side, **kw)
            return post_k(rb)
        def Qu(rb, b, *side, **kw):
            unit(rb, dot_nt, lambda r: (xc, b, r), lambda r: wqc.mx(0, r), side, **kw)
            return post_q(rb, b)
        def loop(n, unroll, body):
            def step(i, carry):
                barrier()
                for u in range(unroll): body(i * unroll + u, u == unroll - 1)
                return carry
            if unroll == n: step(0, 0)
            else: lax.fori_loop(0, n // unroll, step, 0)
            barrier()
        A, B, E = rings
        on = lambda k: only is None or k in only

        wait(('x', 0), ('wg', 0), ('wu', 0))
        run(merge(x_ops(0), w1_ops(0)))
        wait('gw', ('x', 1))
        if on(0):
            p = Fu(A, 0, 0, x_ops(1), gate(0), tail=6)
        wait(('wg', 1), ('wu', 1), ('x', 2)); barrier()
        if on(0):
            p = Fu(B, 1, 0, p, w1_ops(1), tail=2)
            w = x_ops(2)
            p = Fu(A, 0, 1, gate(1) + p, part(w, 0, 2), tail=6)
        wait(('x', 3), 'wk', ('wg', 2), ('wu', 2)); barrier()
        if on(0):
            p = Fu(B, 1, 1, p, part(w, 1, 2), gate(2), tail=2)
            w = x_ops(3)
            p = Fu(A, 2, 0, p, part(w, 0, 2), transpose(wkr, tk))
            p = Fu(B, 2, 1, p, part(w, 1, 2), gate(3), tail=2)
            p = Fu(A, 3, 0, p, wk_ops())
            p = Fu(E, 3, 1, p, w1_ops(2), tail=6)
        wait(*[(n, g) for g in range(3, 7) for n in ('wg', 'wu')])

        def loop1(b, last):
            first = b == 0
            p = post_f(B if not isinstance(b, int) or b else E, jnp.where(first, 3, b - 1) if not isinstance(b, int) else (b - 1) % 4,
                       jnp.where(first, 1, 2) if not isinstance(b, int) else (1 if first else 2))
            p = Ku(A, b, p, w1_ops(3, [2 * b, 2 * b + 1]))
            Fu(B, b, 2, p + pk_ops(b), tail=6 * last)
        def loop1(b, last):
            p = post_f(E, (b + 3) % 4, 1 + jnp.minimum(b, 1) if not isinstance(b, int) else 1 + min(b, 1))
            p = Ku(A, b, p, w1_ops(3, [2 * b, 2 * b + 1]))
            Fu(E, b, 2, p + pk_ops(b), tail=6 * last)
        if on(1): loop(NB, U1, loop1)

        wait('wq', 'wv', 'wo', 'wd')
        if on(2):
            emit = spread(merge(post_f(E, 3, 2) + z_lanes() + transpose(wqr, tq) + z_rows() + wq_ops(), w1_ops(4), w1_ops(5), w1_ops(6), w2_tail()), 196)
            wide_unit(lambda r: [(pkc, b, r) for b in range(4)], lambda r: cat([xc.mx(b, L2R[r // 7] * 7 + L2R[r % 7]) for b in range(4)], 0),
                      None, lambda a: emit, lambda i, j, v: pb.st(0, i, 0, v, col=j))
            p = Fu(A, 0, 3, w2_ops(0))
            hr = lax.broadcasted_iota(jnp.int32, (T, T), 0) // DH
            hl = lax.broadcasted_iota(jnp.int32, (T, T), 1) // DH
            kv = [jnp.where(hr == hl, dot(pb.ref[0, pl.ds(C + j * T, T), :], wv_v[:, ts(j)]), 0.0).astype(bf16) for j in range(4)]
            w = w2_ops(1)
            p = Fu(B, 1, 3, p, part(w, 0, 2))
            for j in range(4):
                w2 = dot(kv[j], wo_v[ts(j), :])
                for n in range(4): st_heads(tw, n, j, w2[:, ts(n)])
            p = Fu(A, 2, 3, p, part(w, 1, 2))
            p = Fu(E, 3, 3, p, w2_ops(3), tail=6)

        def loop2(b, last):
            p = post_f(E, (b + 3) % 4, 3 + 3 * jnp.minimum(b, 1) if not isinstance(b, int) else 3 + 3 * min(b, 1))
            wcell = lambda k, n, c: wdr.ld(0, 8 + k, c, col=n)
            p = Qu(A, b, p, operands(RHS, wcell, lambda r, c, v: w2c.st(0, r * 4 + 2, c, v), [wdr], w2c, 37, [2 * b, 2 * b + 1]))
            p = Fu(B, b, 4, p)
            p = Fu(A, b, 5, p, q_norm(b))
            Fu(E, b, 6, p, tail=6 * last)
        if on(3): loop(NB, U2, loop2)
        run(post_f(E, 3, 6) + h_ops(0, OORDER[0]))

        def ocp(b):
            return pltpu.make_async_copy(rows(ob, 4 * T, b), o_h.at[ds(b * 4 * T, 4 * T, T)], osem.at[b])
        def loop3(b, last):
            wide_unit(lambda r: [(hc, 0, r * 4 + s) for s in range(4)], lambda r: w2c.mx(0, r * 4, 4 * T),
                      lambda r1, i2, j2: ([(hc, 0, 196 + r1 * 2 + i2)], w2c.mx(0, 196 + r1 * 2 + j2)),
                      lambda a: spread(h_ops(b if a < 6 else (b + 1) % NB, OORDER[(a + 1) % 7]), 32 - lag),
                      lambda i, j, v: ob.st(b, i, 0, v, col=j))
            if last:
                for u in range(U3): ocp(b - u).start()
        if on(4):
            loop(NB, U3, loop3)
            for b in range(NB): ocp(b).wait()

    def fn(A_x, A_wqkv, A_wo, B_x, B_w_gate, B_w_up, B_w_down, gate_w):
        anyspec = pl.BlockSpec(memory_space=pl.ANY)
        V = pltpu.VMEM
        B = lambda slots, tiles, dt, lanes=T: V((slots, C + tiles * T, lanes), dt)
        out = pl.pallas_call(
            kernel,
            in_specs=[anyspec] * 7,
            out_specs=anyspec,
            out_shape=jax.ShapeDtypeStruct((S, D), bf16),
            scratch_shapes=[
                V((D, D), bf16), V((D, D), bf16), V((D,), bf16),
                B(4, 4, bf16, D), B(1, 4, bf16, D), B(1, 4, bf16, D), B(7, 4, bf16, 2 * T), B(7, 4, bf16, 2 * T), B(1, 14, bf16, D),
                B(4, 4, bf16, D), B(1, 4, bf16, D), B(4, 4, f32), B(4, 4, f32), B(1, 1, f32), B(4, 4, f32),
                B(4, 49, bf16), B(7, 49, bf16), B(1, 49, bf16), B(1, 49, bf16), B(4, 49, bf16), B(1, 210, bf16), B(1, 210, bf16),
                B(4, 72, f32), B(1, 16, f32), B(4, 5, f32), B(4, 5, f32), B(4, 5, f32),
                B(1, 28, f32), B(1, 28, f32), B(1, 28, f32),
                pltpu.SemaphoreType.DMA((24,)), pltpu.SemaphoreType.DMA((NB,)), pltpu.SemaphoreType.REGULAR,
            ],
            compiler_params=pltpu.CompilerParams(vmem_limit_bytes=120 * 1024 * 1024, flags=flags),
        )(A_x.reshape(S, D), A_wqkv, A_wo, B_w_gate, B_w_up, B_w_down, gate_w)
        return out.reshape(1, S, D)
    return fn


@jax.jit
def pallas_gated_mix__linear_attn_block__swiglu_ffn__prompt_kernel(A_x, A_wqkv, A_wo, B_x, B_w_gate, B_w_up, B_w_down, gate_w):
    return make()(A_x, A_wqkv, A_wo, B_x, B_w_gate, B_w_up, B_w_down, gate_w)
```

```python
import jax
import jax.numpy as jnp
from jax import lax
import jax.experimental.pallas as pl
import jax.experimental.pallas.tpu as pltpu

S, D, F, H, DH = 2048, 512, 1792, 32, 16
T = 128
C = 16
NC = T // C
NB = S // (4 * T)
NG = F // (2 * T)
PITCH = H + 1
UNIT = 49 * T // 4
f32, bf16, u32 = jnp.float32, jnp.bfloat16, jnp.uint32

LHS = (((0, 0, 1), (1, 1, 1)), ((1, 0, 1), (1, 1, 1)), ((0, 0, 1),), ((1, 1, 1),),
       ((0, 0, 1), (0, 1, 1)), ((1, 0, 1), (0, 0, -1)), ((0, 1, 1), (1, 1, -1)))
L2R = (0, 2, 6, 5, 3, 4, 1)
RHS = tuple(LHS[i] for i in L2R)
OUT = (((0, 0, 1), (1, 1, 1)), ((1, 0, 1), (1, 1, -1)), ((0, 1, 1), (1, 1, 1)), ((0, 0, 1), (1, 0, 1)),
       ((0, 1, 1), (0, 0, -1)), ((1, 1, 1),), ((0, 0, 1),))
QUAD = ((0, 0), (0, 1), (1, 0), (1, 1))
ORDER = (1, 3, 6, 0, 4, 2, 5)
WIDE_ORDER = (3, 1, 6, 0, 4, 2, 5)
OUT_INNER_ORDER = (6, 0, 5, 1, 3, 4, 2)
COLD_ORDER = (1, 4, 3, 6, 0, 2, 5)
SLACK, POST_SLACK, SUM_SLACK, TRANSPOSE_SLACK = 256, 320, 448, 512

BUFFERS = dict(
    x=(NB, 4, D, bf16), wq=(1, 4, D, bf16), wk=(1, 4, D, bf16), w1_first=(1, 4, D, bf16),
    w1=(NG, 4, D, bf16), wd=(1, F // T, D, bf16), out=(NB, 4, D, bf16), pkx=(1, 4, D, bf16),
    x_ops=(NB, 49, T, bf16), w1_ops=(NG, 49, T, bf16), wk_ops=(1, 49, T, bf16),
    wq_ops=(1, 49, T, bf16), pk_ops=(NB, 49, T, bf16), w2_ops=(1, 210, T, bf16), h_ops=(1, 210, T, bf16),
    h=(NB, 52, T, f32), h_last=(1, 8, T, f32), pq=(1, 20, T, f32), pk=(NB, 16, T, f32), den=(1, 8, T, f32),
    h_weight=(1, 4, T, f32), pq_weight=(1, 4, T, f32), rows=(2, 1, T, f32), wk_t=(4, 5, T, f32), wq_t=(4, 5, T, f32), w2=(4, 5, T, f32))


def signed_sum(terms):
    sign, acc = terms[0]
    for s, v in terms[1:]:
        if s == sign:
            acc = acc + v
        elif sign > 0:
            acc = acc - v
        else:
            sign, acc = 1, v - acc
    return sign, acc


def combine(terms, block):
    return signed_sum([(s, block(i, j)) for i, j, s in terms])[1]


def quadrants(m):
    return {(0, 0): (m[0] + m[6]) + (m[3] - m[4]), (0, 1): m[2] + m[4],
            (1, 0): m[1] + m[3], (1, 1): (m[0] + m[5]) + (m[2] - m[1])}


def dot(a, b):
    return jnp.dot(a, b, preferred_element_type=f32)


def dot_nt(a, b):
    return lax.dot_general(a, b, (((1,), (1,)), ((), ())), preferred_element_type=f32)


def phi(t):
    return jnp.where(t > 0, t + 1.0, jnp.exp(t)) + 1e-6


def swiglu(gate, up):
    half = 0.5 * gate
    return (half * jnp.tanh(half) + half) * up


def lanes(i, n=1):
    return slice(i * T, (i + n) * T)


def cat(parts, axis):
    return jnp.concatenate(parts, axis=axis) if len(parts) > 1 else parts[0]


def interleave(*lists):
    keyed = [((k + 0.5) / len(l), j, k) for j, l in enumerate(lists) for k in range(len(l))]
    return [lists[j][k] for _, j, k in sorted(keyed)]


def tile_pitch(width, dtype):
    return T + ((8 if dtype == f32 else C) if width == T else 0)


class Buffer:
    def __init__(self, ref, spare):
        self.ref = ref
        self.raw = ref.bitcast(u32) if (ref.dtype, ref.shape[-1]) == (bf16, T) else None
        self.pitch = tile_pitch(ref.shape[-1], ref.dtype)
        self.spare = spare

    def store(self, slot, tile, c, v, col=0):
        self.ref[slot, pl.ds(C + tile * self.pitch + c * C, v.shape[0]), lanes(col)] = v.astype(self.ref.dtype)

    def load(self, slot, tile, c=0, n=C, col=0, cols=1):
        return self.ref[slot, pl.ds(C + tile * self.pitch + c * C, n), lanes(col, cols)].astype(f32)

    def word_rows(self, tile, c, n):
        return pl.ds((C + tile * self.pitch + c * C) // 2, n // 2)

    def words(self, slot, tile, c=0, n=T):
        return self.raw[slot, self.word_rows(tile, c, n), :]

    def operand(self, slot, tile):
        return pltpu.bitcast(self.words(slot, tile), bf16)

    def gate(self, v):
        self.ref[0, pl.ds(self.spare, v.shape[0]), 0:T] = v.astype(self.ref.dtype)

    def token(self):
        if self.raw is not None:
            return self.raw[0, pl.ds(self.spare, 8), :]
        return pltpu.bitcast(self.ref[0, pl.ds(self.spare, 8 if self.ref.dtype == f32 else C), 0:T], u32)


class Task:
    def __init__(self, cost, reads, writes, slack, run, *args):
        self.cost, self.reads, self.writes, self.slack = cost, reads, writes, slack
        self.run = lambda: run(*args)


class Stream:
    def __init__(self, never):
        self.never = never
        self.queue = []
        self.aligning = False
        self.restart()

    def restart(self):
        assert not self.queue
        self.time, self.tiles, self.due, self.recent = 0, 0, [], []

    def host(self, tasks, end, start=0):
        total, spent = sum(t.cost for t in tasks), 0
        for t in tasks:
            self.queue.append((self.time + start + (end - start) * spent // total, t))
            spent += t.cost
        self.queue.sort(key=lambda entry: entry[0])

    def expect(self, buffers, slack):
        self.due += [(self.time + slack, b.token()) for b in buffers]

    def align(self, step):
        old = [m for t, m in self.recent if t <= self.time - T][-4:]
        token = None
        for a, m in enumerate(old):
            if a == 0 or m is not old[a - 1]:
                word = pltpu.bitcast(m[0:8, 0:T], u32)
                token = word if token is None else token | word
        if old:
            self.due += [(self.time + a * step, token) for a in range(4)]

    def product(self, fn, lhs, rhs):
        step = lhs[0].shape[0] // 2
        row = [((a if len(lhs) == 4 else self.tiles + a) % 4) * step // C * 8 for a in range(len(lhs))]
        operands = []
        for a, w in enumerate(lhs):
            tokens = [k for t, k in self.due if t <= self.time + a * step]
            self.due = [entry for entry in self.due if entry[0] > self.time + a * step]
            if tokens:
                token = tokens[0]
                for other in tokens[1:]:
                    token = token | other
                lo, hi = row[a], row[a] + 8
                w = cat([w[i:j] if n != 1 else jnp.where(self.never, token, w[i:j])
                         for n, (i, j) in enumerate(((0, lo), (lo, hi), (hi, w.shape[0]))) if i < j], 0)
            operands.append(pltpu.bitcast(w, bf16))
        m = fn(cat(operands, 1), rhs)
        self.recent = self.recent[-31:] + [(self.time, m)] * len(lhs)
        for a in range(len(lhs)):
            gated, written = [], []
            while self.queue and self.queue[0][0] < self.time + step:
                task = self.queue.pop(0)[1]
                for b in task.reads:
                    if b not in gated:
                        b.gate(m[2 * row[a]:2 * row[a] + 8])
                        gated.append(b)
                task.run()
                written += [(b, task.slack) for b in task.writes if (b, task.slack) not in written]
            for b, slack in written:
                self.expect([b], slack)
            self.time += step
        self.tiles += len(lhs)
        return m


def kernel(x_hbm, wqkv_hbm, wo_hbm, wg_hbm, wu_hbm, wd_hbm, gw_hbm, out_hbm,
           wv_ref, wo_ref, gw_ref, zero_ref, in_sems, out_sem, *refs):
    ref = dict(zip(BUFFERS, refs))
    copies = {}

    def fetch(name, src, dst):
        copies[name] = pltpu.make_async_copy(src, dst, in_sems.at[len(copies)])
        copies[name].start()

    def fetch_x(name, row, n):
        fetch(name, x_hbm.at[pl.ds(row, n)], ref['x'].at[row // (4 * T), pl.ds(C + row % (4 * T), n)])

    def fetch_w1(name, col, n):
        dst = ref['w1' if col >= 2 * T else 'w1_first']
        for u, src in enumerate((wg_hbm, wu_hbm)):
            fetch((name, u), src.at[:, pl.ds(col, n)],
                  dst.at[col // (2 * T), pl.ds(C, D), pl.ds(u * 2 * T + col % (2 * T), n)])

    fetch_x('x0a', 0, 2 * T)
    fetch_w1('w0a', 0, T)
    fetch_w1('w0b', T, T)
    fetch_x('x0b', 2 * T, 2 * T)
    fetch_x('x1', 4 * T, 4 * T)
    fetch_x('x2', 8 * T, 4 * T)
    fetch_x('x3', 12 * T, 4 * T)
    fetch_w1(1, 2 * T, 2 * T)
    fetch('gw', gw_hbm, gw_ref)
    fetch('wk', wqkv_hbm.at[:, pl.ds(D, D)], ref['wk'].at[0, pl.ds(C, D)])
    for g in range(2, NG):
        fetch_w1(g, g * 2 * T, 2 * T)
    fetch('wq', wqkv_hbm.at[:, pl.ds(0, D)], ref['wq'].at[0, pl.ds(C, D)])
    fetch('wv', wqkv_hbm.at[:, pl.ds(2 * D, D)], wv_ref)
    fetch('wo', wo_hbm, wo_ref)
    fetch('wd', wd_hbm, ref['wd'].at[0, pl.ds(C, F)])

    @pl.loop(0, 2)
    def _(i):
        zero_ref[i] = 0
    zero = zero_ref[1]
    spare = pl.multiple_of(zero * C, C)
    buffers = [Buffer(r, spare) for r in refs]
    for b in buffers:
        b.gate(jnp.zeros((C, T), f32))
    (x, wq, wk, w1_first, w1, wd, out, pkx, x_ops, w1_ops, wk_ops, wq_ops, pk_ops, w2_ops, h_ops,
     h, h_last, pq, pk, den, h_weight, pq_weight, rows, wk_t, wq_t, w2) = buffers
    stream = Stream(zero != 0)

    def wait(*names):
        for name in names:
            copies[name].wait()
        stream.restart()

    def sums(table, block, store, reads, writes, cost, outer=ORDER):
        def run(r1, c):
            inner = {q: combine(table[r1], lambda i, j: block(2 * i + q[0], 2 * j + q[1], c)) for q in QUAD}
            for r2 in range(7):
                store(r1 * 7 + r2, c, combine(table[r2], lambda i, j: inner[i, j]))
        return [Task(cost[len(table[r1]) - 1], reads, writes, SLACK, run, r1, c) for c in range(NC) for r1 in outer]

    from_bf16, from_f32 = (25, 41), (25, 32)

    def x_sums(b, outer=ORDER):
        return sums(LHS, lambda i, j, c: x.load(b, i, c, col=j),
                    lambda r, c, v: x_ops.store(b, r, c, v), [x], [x_ops], from_bf16, outer)

    def w1_sums(g, outer=ORDER):
        src = w1 if g else w1_first
        return sums(RHS, lambda k, n, c: src.load(g, k, c, col=n % 2 * 2 + n // 2),
                    lambda r, c, v: w1_ops.store(g, r, c, v), [src], [w1_ops], from_bf16, outer)

    def store_head_minor(dst, slot, head, v):
        for n in range(v.shape[0] // DH):
            dst.ref[slot, pl.ds(C + head + n, DH, stride=PITCH), :] = v[n * DH:(n + 1) * DH]

    def load_head_minor(src, slot, tile, c):
        j = tile * T + c * C
        return src.ref[slot, pl.ds(C + j // H * PITCH + j % H, C), :]

    def transposes(src, dst, cost, store):
        def run(k, j):
            store(k, j, src.load(0, k, 0, T, col=j).T)
        return [Task(cost, [src], [dst], TRANSPOSE_SLACK, run, k, j) for k in range(4) for j in range(4)]

    def wk_sums():
        return sums(RHS, wk_t.load, lambda r, c, v: wk_ops.store(0, r, c, v), [wk_t], [wk_ops], (32, 38))

    def wq_sums():
        return sums(RHS, lambda k, j, c: load_head_minor(wq_t, k, j, c),
                    lambda r, c, v: wq_ops.store(0, r, c, v), [wq_t], [wq_ops], from_f32)

    def pk_sums(r1):
        return interleave(*[
            sums(LHS, lambda j, i, c, b=b: pk.load(b, j * 4 + i, c),
                 lambda r, c, v, b=b: pk_ops.store(b, r, c, v), [pk], [pk_ops], from_f32, [r1])
            for b in range(NB)])

    def z_columns():
        def run(j, c):
            p = [(pk.load(b, j * 4, c) + pk.load(b, j * 4 + 1, c))
                 + (pk.load(b, j * 4 + 2, c) + pk.load(b, j * 4 + 3, c)) for b in range(NB)]
            z = jnp.sum((p[0] + p[1]) + (p[2] + p[3]), axis=1, keepdims=True)
            store_head_minor(wk_t, 0, j * NC + c, jnp.broadcast_to(z, (C, T)))
        return [Task(35, [pk], [wk_t], SUM_SLACK, run, j, c) for j in range(4) for c in range(NC)]

    def z_rows():
        def run(j):
            rows.store(1, 0, j, cat([load_head_minor(wk_t, 0, j, c) for c in range(NC)], 0).T[0:C])
        return [Task(30, [wk_t], [rows], SUM_SLACK, run, j) for j in range(4)]

    def w2_sums(s):
        store = lambda r, c, v: w2_ops.store(0, s * 49 + r, c, v)
        if s == 3:
            return sums(RHS, lambda k, n, c: load_head_minor(w2, n, k, c), store, [w2], [w2_ops], from_f32)
        return sums(RHS, lambda k, n, c: wd.load(0, 4 * s + k, c, col=n), store, [wd], [w2_ops], from_bf16)

    def w2_last_sums():
        def run(n2, c):
            v = {(k, n1): wd.load(0, 12 + k, c, col=2 * n1 + n2) for k, n1 in QUAD}
            for r1 in range(7):
                w2_ops.store(0, 196 + r1 * 2 + n2, c, combine(RHS[r1], lambda i, j: v[i, j]))
        return [Task(25, [wd], [w2_ops], SLACK, run, n2, c) for n2 in range(2) for c in range(NC)]

    def h_sums(b, r1):
        tasks = []
        for s in range(4):
            src, slot, n, first, weight = (pq, 0, 5, 0, pq_weight) if s == 3 else (h, b, 13, 4 * s, h_weight)

            def block(i, k, c, src=src, slot=slot, n=n, first=first, weight=weight):
                return src.load(slot, i * n + first + k, c) * weight.load(0, i, c)
            tasks += sums(LHS, block, lambda r, c, v, s=s: h_ops.store(0, s * 49 + r, c, v),
                          [src], [h_ops], from_bf16, [r1])
        return tasks

    def h_last_sums():
        def run(i2, c):
            v = {(i1, k): h_last.load(0, (2 * i1 + i2) * 2 + k, c) * h_weight.load(0, 2 * i1 + i2, c) for i1, k in QUAD}
            for r1 in range(7):
                h_ops.store(0, 196 + r1 * 2 + i2, c, combine(LHS[r1], lambda i, j: v[i, j]))
        return [Task(25, [h_last], [h_ops], SLACK, run, i2, c) for c in range(NC) for i2 in range(2)]

    def ffn_weights(b):
        def run(i, c):
            p = [x.load(b, i, c, col=j) * rows.load(0, 0, j) for j in range(4)]
            t = jnp.sum((p[0] + p[1]) + (p[2] + p[3]), axis=1, keepdims=True)
            h_weight.store(0, i, c, jnp.broadcast_to(0.5 - 0.5 * jnp.tanh(t), (C, T)))
        return [Task(30, [x], [h_weight], SUM_SLACK, run, i, c) for c in range(NC) for i in range(4)]

    def attention_weights():
        def run(i, c):
            t = den.load(0, i * 2, c) + den.load(0, i * 2 + 1, c)
            t = t + pltpu.roll(t, 2 * H, 1)
            t = t + pltpu.roll(t, H, 1)
            pq_weight.store(0, i, c, (1.0 - h_weight.load(0, i, c)) / (t + 1e-6))
        return [Task(30, [den], [pq_weight], SUM_SLACK + 128, run, i, c) for c in range(NC) for i in range(4)]

    def strassen(fn, lhs, rhs, n, order, finish, writes, extra=None, before=None):
        if stream.aligning and not extra:
            stream.align(n // 4)
        for c in range(0, NC, n // C):
            acc, seen = {}, dict.fromkeys(QUAD, 0)
            for a, r1 in enumerate(order):
                if before:
                    before(a)
                inner = quadrants({r2: stream.product(fn, lhs(r1 * 7 + r2, c, n), rhs(r1 * 7 + r2))
                                   for r2 in (OUT_INNER_ORDER if extra else ORDER)})
                if extra:
                    inner = {q: inner[q] + extra(r1, *q) for q in QUAD}
                for i1, j1, sign in OUT[r1]:
                    for q in QUAD:
                        new = (sign, inner[q])
                        acc[i1, j1, q] = signed_sum([acc[i1, j1, q], new]) if seen[i1, j1] else new
                    seen[i1, j1] += 1
                    if seen[i1, j1] == (4 if i1 == j1 else 2):
                        finish(i1, j1, c, {q: acc[i1, j1, q][1] for q in QUAD})
                        stream.expect(writes, POST_SLACK)

    def ffn_plain(quarters, cols):
        for j in cols:
            for i in quarters:
                def gemm(col):
                    w = pltpu.bitcast(x.ref[0, pl.ds(C + i * T, T), :], u32)
                    return stream.product(dot, [w[:, lanes(k)] for k in range(4)],
                                          w1_first.ref[0, pl.ds(C, D), lanes(col)])
                h.store(0, i * 13 + j, 0, swiglu(gemm(j), gemm(2 + j)))
                stream.expect([h], POST_SLACK)

    def ffn(b, g, n=64, order=ORDER):
        def finish(i1, j1, c, v):
            for i2 in range(2):
                i, act = 2 * i1 + i2, swiglu(v[i2, 0], v[i2, 1])
                if g == NG - 1:
                    h_last.store(0, i * 2 + j1, c, act)
                else:
                    h.store(b, i * 13 + 2 * g + j1, c, act)
        strassen(dot, lambda r, c, n: [x_ops.words(b, r, c, n)],
                 lambda r: w1_ops.operand(g, r), n, order, finish, [h_last if g == NG - 1 else h])

    def keys(b):
        def finish(i1, j1, c, v):
            for i2, j2 in QUAD:
                pk.store(b, (2 * j1 + j2) * 4 + 2 * i1 + i2, c, phi(v[i2, j2]))
        strassen(dot_nt, lambda r, c, n: [wk_ops.words(0, r, c, n)], lambda r: x_ops.operand(b, r),
                 64, ORDER, finish, [pk])

    def queries(b):
        def finish(i1, j1, c, v):
            z = [cat([rows.load(1, 0, 2 * j1 + j2)] * 4, 0) for j2 in range(2)]
            for i2 in range(2):
                i, p = 2 * i1 + i2, [phi(v[i2, j2]) for j2 in range(2)]
                for j2 in range(2):
                    pq.store(0, i * 5 + 2 * j1 + j2, c, p[j2])
                den.store(0, i * 2 + j1, c, p[0] * z[0] + p[1] * z[1])
        strassen(dot_nt, lambda r, c, n: [x_ops.words(b, r, c, n)], lambda r: wq_ops.operand(0, r),
                 64, ORDER, finish, [pq, den])

    def store_quadrant(dst, slot, i1, j1, c, v):
        for i2, j2 in QUAD:
            dst.store(slot, 2 * i1 + i2, c, v[i2, j2], col=2 * j1 + j2)

    def out_copy(b, i1, j1):
        return pltpu.make_async_copy(
            out.ref.at[b, pl.ds(C + i1 * 2 * T, 2 * T), pl.ds(j1 * 2 * T, 2 * T)],
            out_hbm.at[pl.ds(pl.multiple_of((b * 4 + i1 * 2) * T, T), 2 * T), pl.ds(j1 * 2 * T, 2 * T)], out_sem)

    def ungated(tasks):
        return [Task(t.cost, [], t.writes, t.slack, t.run) for t in tasks]

    def run_now(tasks):
        for task in tasks:
            task.run()

    w0, x0 = w1_sums(0), x_sums(0, (1, 3, 6, 0, 5))
    wait('x0a', ('w0a', 0), ('w0a', 1))
    stream.host(ungated(x_sums(0, (2, 4))), 256)
    ffn_plain((0, 1), (0,))
    wait(('w0b', 0), ('w0b', 1))
    stream.host(ungated(w0[:10]), 320)
    ffn_plain((0, 1), (1,))
    wait('x0b')
    stream.host(ungated(w0[10:] + x0[:8]), 832)
    ffn_plain((2, 3), (0, 1))
    wait('x1')
    tasks = x_sums(1)
    run_now(tasks[:14])
    stream.host(tasks[14:], UNIT * 5 // 8)
    stream.host(x0[8:22], UNIT - T, UNIT * 5 // 8)
    ffn(1, 0, 32)
    wait('x2', 'x3')
    tasks = x_sums(2)
    run_now(tasks[:14])
    stream.host(tasks[14:], UNIT * 5 // 8)
    stream.host(x_sums(3) + x0[22:], 2 * UNIT - T, UNIT * 5 // 8)
    ffn(2, 0, 32)
    ffn(3, 0, 32)

    wait((1, 0), (1, 1), 'gw', 'wk', (2, 0), (2, 1))
    tasks = sum([w1_sums(1, [r1]) for r1 in COLD_ORDER], [])
    run_now(tasks[:17])
    stream.host(tasks[17:], 1050)
    tasks = w1_sums(2)
    stream.host(transposes(wk, wk_t, 70, lambda k, j, v: wk_t.store(k, j, 0, v)) + tasks[:14] + wk_sums(),
                4 * UNIT - SLACK, UNIT - SLACK)
    ffn(0, 1, T, COLD_ORDER)
    for b in range(1, NB):
        ffn(b, 1)
    stream.host(tasks[14:], 4 * UNIT - POST_SLACK)
    for b in range(NB):
        keys(b)
    half_gw = 0.5 * gw_ref[...].astype(f32).reshape(1, D)
    for j in range(4):
        rows.store(0, 0, j, jnp.broadcast_to(half_gw[:, lanes(j)], (C, T)))

    wait(*[(g, u) for g in range(3, NG) for u in range(2)], 'wq', 'wv', 'wo', 'wd')
    stream.aligning = True
    tasks = w1_sums(3) + w1_sums(4) + w1_sums(5) + w1_sums(6)
    stream.host(tasks[:35] + pk_sums(WIDE_ORDER[0]) + pk_sums(WIDE_ORDER[1]), 2 * UNIT)
    ffn(0, 2)
    ffn(1, 2)
    stream.host(interleave(sum([pk_sums(r1) for r1 in WIDE_ORDER[2:]], []) + z_columns(),
                           tasks[35:147] + ffn_weights(0) + w2_last_sums()), 4 * UNIT)
    strassen(dot, lambda r, c, n: [pk_ops.words(b, r, c, n) for b in range(NB)],
             lambda r: cat([x_ops.operand(b, L2R[r // 7] * 7 + L2R[r % 7]) for b in range(NB)], 0),
             T, WIDE_ORDER, lambda *a: store_quadrant(pkx, 0, *a), [pkx])
    stream.host(transposes(wq, wq_t, 60, lambda k, j, v: store_head_minor(wq_t, k, j * NC, v)) + z_rows()
                + wq_sums() + tasks[147:] + sum([w2_sums(s) for s in range(4)], []), 10 * UNIT - 224, 64)
    ffn(2, 2)
    same_head = (lax.broadcasted_iota(jnp.int32, (T, T), 0) // DH
                 == lax.broadcasted_iota(jnp.int32, (T, T), 1) // DH)
    kv = [jnp.where(same_head, dot(pkx.ref[0, pl.ds(C + j * T, T), :], wv_ref[:, lanes(j)]), 0.0).astype(bf16)
          for j in range(4)]
    ffn(3, 2)
    for j in range(4):
        v = dot(kv[j], wo_ref[lanes(j), :])
        for n in range(4):
            store_head_minor(w2, n, j * NC, v[:, lanes(n)])
    stream.recent = []
    stream.expect([w2], SLACK)
    for g in (3, 4):
        for b in range(NB):
            ffn(b, g)

    @pl.loop(0, NB)
    def _(b):
        stream.restart()
        queries(b)
        stream.host(attention_weights() + h_sums(b, WIDE_ORDER[0]), 2 * UNIT - 288)
        ffn(b, 5)
        ffn(b, 6)

        def before(a):
            if a < 6:
                stream.host((h_last_sums() if a == 0 else []) + h_sums(b, WIDE_ORDER[a + 1]), 8 * T - 192)
            else:
                stream.host(ffn_weights((b + 1) % NB), 8 * T - SUM_SLACK)

        def finish(i1, j1, c, v):
            store_quadrant(out, b, i1, j1, c, v)
            out_copy(b, i1, j1).start()

        strassen(dot, lambda r, c, n: [h_ops.words(0, s * 49 + r, c, n) for s in range(4)],
                 lambda r: cat([w2_ops.operand(0, s * 49 + r) for s in range(4)], 0),
                 T, WIDE_ORDER, finish, [out], before=before,
                 extra=lambda r1, i2, j2: stream.product(dot, [h_ops.words(0, 196 + r1 * 2 + i2)],
                                                         w2_ops.operand(0, 196 + r1 * 2 + j2)))
        stream.restart()

    for b in range(NB):
        for q in QUAD:
            out_copy(b, *q).wait()


@jax.jit
def pallas_gated_mix__linear_attn_block__swiglu_ffn__prompt_kernel(
    A_x: jax.Array,
    A_wqkv: jax.Array,
    A_wo: jax.Array,
    B_x: jax.Array,
    B_w_gate: jax.Array,
    B_w_up: jax.Array,
    B_w_down: jax.Array,
    gate_w: jax.Array,
):
    del B_x

    def scratch(slots, tiles, width, dtype):
        n = C + tiles * tile_pitch(width, dtype)
        return pltpu.VMEM((slots, -(-n // 64) * 64, width), dtype)

    hbm = pl.BlockSpec(memory_space=pl.ANY)
    result = pl.pallas_call(
        kernel,
        in_specs=[hbm] * 7,
        out_specs=hbm,
        out_shape=jax.ShapeDtypeStruct((S, D), bf16),
        scratch_shapes=[
            pltpu.VMEM((D, D), bf16), pltpu.VMEM((D, D), bf16), pltpu.VMEM((D,), bf16),
            pltpu.SMEM((2,), jnp.int32), pltpu.SemaphoreType.DMA((27,)), pltpu.SemaphoreType.DMA,
            *[scratch(*spec) for spec in BUFFERS.values()]],
        compiler_params=pltpu.CompilerParams(
            vmem_limit_bytes=112 * 1024 * 1024, disable_bounds_checks=True, disable_semaphore_checks=True),
    )(A_x.reshape(S, D), A_wqkv, A_wo, B_w_gate, B_w_up, B_w_down, gate_w)
    return result.reshape(1, S, D)
```

```python
import jax
import jax.numpy as jnp
from jax import lax
import jax.experimental.pallas as pl
import jax.experimental.pallas.tpu as pltpu

S, D, F, H, DH = 2048, 512, 1792, 32, 16
T = 128
C = 16
NC = T // C
NB = S // (4 * T)
NG = F // (2 * T)
PITCH = H + 1
UNIT = 49 * T // 4
f32, bf16, u32 = jnp.float32, jnp.bfloat16, jnp.uint32

LHS = (((0, 0, 1), (1, 1, 1)), ((1, 0, 1), (1, 1, 1)), ((0, 0, 1),), ((1, 1, 1),),
       ((0, 0, 1), (0, 1, 1)), ((1, 0, 1), (0, 0, -1)), ((0, 1, 1), (1, 1, -1)))
L2R = (0, 2, 6, 5, 3, 4, 1)
RHS = tuple(LHS[i] for i in L2R)
OUT = (((0, 0, 1), (1, 1, 1)), ((1, 0, 1), (1, 1, -1)), ((0, 1, 1), (1, 1, 1)), ((0, 0, 1), (1, 0, 1)),
       ((0, 1, 1), (0, 0, -1)), ((1, 1, 1),), ((0, 0, 1),))
QUAD = ((0, 0), (0, 1), (1, 0), (1, 1))
ORDER = (1, 3, 6, 0, 4, 2, 5)
WIDE_ORDER = (3, 1, 6, 0, 4, 2, 5)
OUT_INNER_ORDER = (6, 0, 5, 1, 3, 4, 2)
COLD_ORDER = (1, 4, 3, 6, 0, 2, 5)
SLACK, POST_SLACK, SUM_SLACK, TRANSPOSE_SLACK = 256, 320, 448, 512

BUFFERS = dict(
    x=(NB, 4, D, bf16), wq=(1, 4, D, bf16), wk=(1, 4, D, bf16), w1_first=(1, 4, D, bf16),
    w1=(NG, 4, D, bf16), wd=(1, F // T, D, bf16), out=(NB, 4, D, bf16), pkx=(1, 4, D, bf16),
    x_ops=(NB, 49, T, bf16), w1_ops=(NG, 49, T, bf16), wk_ops=(1, 49, T, bf16),
    wq_ops=(1, 49, T, bf16), pk_ops=(NB, 49, T, bf16), w2_ops=(1, 210, T, bf16), h_ops=(1, 210, T, bf16),
    h=(NB, 52, T, f32), h_last=(1, 8, T, f32), pq=(1, 20, T, f32), pk=(NB, 16, T, f32), den=(1, 8, T, f32),
    h_weight=(1, 4, T, f32), pq_weight=(1, 4, T, f32), rows=(2, 1, T, f32),
    wk_t=(4, 5, T, f32), wq_t=(4, 5, T, f32), w2=(4, 5, T, f32))


def signed_sum(terms):
    sign, acc = terms[0]
    for s, v in terms[1:]:
        if s == sign:
            acc = acc + v
        elif sign > 0:
            acc = acc - v
        else:
            sign, acc = 1, v - acc
    return sign, acc


def combine(terms, block):
    return signed_sum([(s, block(i, j)) for i, j, s in terms])[1]


def quadrants(m):
    return {(0, 0): (m[0] + m[6]) + (m[3] - m[4]), (0, 1): m[2] + m[4],
            (1, 0): m[1] + m[3], (1, 1): (m[0] + m[5]) + (m[2] - m[1])}


def dot(a, b):
    return jnp.dot(a, b, preferred_element_type=f32)


def dot_nt(a, b):
    return lax.dot_general(a, b, (((1,), (1,)), ((), ())), preferred_element_type=f32)


def phi(t):
    return jnp.where(t > 0, t + 1.0, jnp.exp(t)) + 1e-6


def swiglu(gate, up):
    half = 0.5 * gate
    return (half * jnp.tanh(half) + half) * up


def lanes(i):
    return slice(i * T, (i + 1) * T)


def cat(parts, axis):
    return jnp.concatenate(parts, axis=axis) if len(parts) > 1 else parts[0]


def interleave(*lists):
    keyed = [((k + 0.5) / len(l), j, k) for j, l in enumerate(lists) for k in range(len(l))]
    return [lists[j][k] for _, j, k in sorted(keyed)]


def tile_pitch(width, dtype):
    return T + ((8 if dtype == f32 else C) if width == T else 0)


class Buffer:
    def __init__(self, ref, spare):
        self.ref = ref
        self.raw = ref.bitcast(u32) if (ref.dtype, ref.shape[-1]) == (bf16, T) else None
        self.pitch = tile_pitch(ref.shape[-1], ref.dtype)
        self.spare = spare

    def store(self, slot, tile, c, v, col=0):
        self.ref[slot, pl.ds(C + tile * self.pitch + c * C, v.shape[0]), lanes(col)] = v.astype(self.ref.dtype)

    def load(self, slot, tile, c=0, n=C, col=0):
        return self.ref[slot, pl.ds(C + tile * self.pitch + c * C, n), lanes(col)].astype(f32)

    def words(self, slot, tile, c=0, n=T):
        return self.raw[slot, pl.ds((C + tile * self.pitch + c * C) // 2, n // 2), :]

    def operand(self, slot, tile):
        return pltpu.bitcast(self.words(slot, tile), bf16)

    def gate(self, v):
        self.ref[0, pl.ds(self.spare, v.shape[0]), 0:T] = v.astype(self.ref.dtype)

    def token(self):
        if self.raw is not None:
            return self.raw[0, pl.ds(self.spare, 8), :]
        return pltpu.bitcast(self.ref[0, pl.ds(self.spare, 8 if self.ref.dtype == f32 else C), 0:T], u32)


class Task:
    def __init__(self, cost, reads, writes, slack, run, *args):
        self.cost, self.reads, self.writes, self.slack = cost, reads, writes, slack
        self.run = lambda: run(*args)


class Stream:
    def __init__(self, never):
        self.never = never
        self.queue = []
        self.aligning = False
        self.restart()

    def restart(self):
        assert not self.queue
        self.time, self.tiles, self.due, self.recent = 0, 0, [], []

    def host(self, tasks, end, start=0):
        total, spent = sum(t.cost for t in tasks), 0
        for t in tasks:
            self.queue.append((self.time + start + (end - start) * spent // total, t))
            spent += t.cost
        self.queue.sort(key=lambda entry: entry[0])

    def expect(self, buffers, slack):
        self.due += [(self.time + slack, b.token()) for b in buffers]

    def align(self, step):
        old = [m for t, m in self.recent if t <= self.time - T][-4:]
        token = None
        for a, m in enumerate(old):
            if a == 0 or m is not old[a - 1]:
                word = pltpu.bitcast(m[0:8, 0:T], u32)
                token = word if token is None else token | word
        if old:
            self.due += [(self.time + a * step, token) for a in range(4)]

    def product(self, fn, lhs, rhs):
        step = lhs[0].shape[0] // 2
        row = [((a if len(lhs) == 4 else self.tiles + a) % 4) * step // C * 8 for a in range(len(lhs))]
        operands = []
        for a, w in enumerate(lhs):
            tokens = [k for t, k in self.due if t <= self.time + a * step]
            self.due = [entry for entry in self.due if entry[0] > self.time + a * step]
            if tokens:
                token = tokens[0]
                for other in tokens[1:]:
                    token = token | other
                lo, hi = row[a], row[a] + 8
                w = cat([w[i:j] if n != 1 else jnp.where(self.never, token, w[i:j])
                         for n, (i, j) in enumerate(((0, lo), (lo, hi), (hi, w.shape[0]))) if i < j], 0)
            operands.append(pltpu.bitcast(w, bf16))
        m = fn(cat(operands, 1), rhs)
        self.recent = self.recent[-31:] + [(self.time, m)] * len(lhs)
        for a in range(len(lhs)):
            gated, written = [], []
            while self.queue and self.queue[0][0] < self.time + step:
                task = self.queue.pop(0)[1]
                for b in task.reads:
                    if b not in gated:
                        b.gate(m[2 * row[a]:2 * row[a] + 8])
                        gated.append(b)
                task.run()
                written += [(b, task.slack) for b in task.writes if (b, task.slack) not in written]
            for b, slack in written:
                self.expect([b], slack)
            self.time += step
        self.tiles += len(lhs)
        return m


def kernel(x_hbm, wqkv_hbm, wo_hbm, wg_hbm, wu_hbm, wd_hbm, gw_hbm, out_hbm,
           wv_ref, wo_ref, gw_ref, zero_ref, in_sems, out_sems, *refs):
    ref = dict(zip(BUFFERS, refs))
    copies = {}

    def fetch(name, src, dst):
        copies[name] = pltpu.make_async_copy(src, dst, in_sems.at[len(copies)])
        copies[name].start()

    def fetch_x(name, row, n):
        fetch(name, x_hbm.at[pl.ds(row, n)], ref['x'].at[row // (4 * T), pl.ds(C + row % (4 * T), n)])

    def fetch_w1(name, col, n):
        dst = ref['w1' if col >= 2 * T else 'w1_first']
        for u, src in enumerate((wg_hbm, wu_hbm)):
            fetch((name, u), src.at[:, pl.ds(col, n)],
                  dst.at[col // (2 * T), pl.ds(C, D), pl.ds(u * 2 * T + col % (2 * T), n)])

    fetch_x('x0a', 0, T)
    fetch_w1('w0a', 0, T)
    fetch_x('x0b', T, 2 * T)
    fetch_x('x0c', 3 * T, T)
    fetch_w1('w0b', T, T)
    fetch_x('x1', 4 * T, 4 * T)
    fetch_x('x2', 8 * T, 4 * T)
    fetch_x('x3', 12 * T, 4 * T)
    fetch_w1(1, 2 * T, 2 * T)
    fetch('gw', gw_hbm, gw_ref)
    fetch('wk', wqkv_hbm.at[:, pl.ds(D, D)], ref['wk'].at[0, pl.ds(C, D)])
    for g in range(2, NG):
        fetch_w1(g, g * 2 * T, 2 * T)
    fetch('wq', wqkv_hbm.at[:, pl.ds(0, D)], ref['wq'].at[0, pl.ds(C, D)])
    fetch('wv', wqkv_hbm.at[:, pl.ds(2 * D, D)], wv_ref)
    fetch('wo', wo_hbm, wo_ref)
    fetch('wd', wd_hbm, ref['wd'].at[0, pl.ds(C, F)])

    @pl.loop(0, 2)
    def _(i):
        zero_ref[i] = 0
    zero = zero_ref[1]
    spare = pl.multiple_of(zero * C, C)
    buffers = [Buffer(r, spare) for r in refs]
    for b in buffers:
        b.gate(jnp.zeros((C, T), f32))
    (x, wq, wk, w1_first, w1, wd, out, pkx, x_ops, w1_ops, wk_ops, wq_ops, pk_ops, w2_ops, h_ops,
     h, h_last, pq, pk, den, h_weight, pq_weight, rows, wk_t, wq_t, w2) = buffers
    stream = Stream(zero != 0)

    def wait(*names):
        for name in names:
            copies[name].wait()
        stream.restart()

    def sums(table, block, store, reads, writes, cost, outer=ORDER):
        def run(r1, c):
            inner = {q: combine(table[r1], lambda i, j: block(2 * i + q[0], 2 * j + q[1], c)) for q in QUAD}
            for r2 in range(7):
                store(r1 * 7 + r2, c, combine(table[r2], lambda i, j: inner[i, j]))
        return [Task(cost[len(table[r1]) - 1], reads, writes, SLACK, run, r1, c) for c in range(NC) for r1 in outer]

    from_bf16, from_f32 = (25, 41), (25, 32)

    def x_sums(b, outer=ORDER):
        return sums(LHS, lambda i, j, c: x.load(b, i, c, col=j),
                    lambda r, c, v: x_ops.store(b, r, c, v), [x], [x_ops], from_bf16, outer)

    def w1_sums(g, outer=ORDER):
        src = w1 if g else w1_first
        return sums(RHS, lambda k, n, c: src.load(g, k, c, col=n % 2 * 2 + n // 2),
                    lambda r, c, v: w1_ops.store(g, r, c, v), [src], [w1_ops], from_bf16, outer)

    def store_head_minor(dst, slot, head, v):
        for n in range(v.shape[0] // DH):
            dst.ref[slot, pl.ds(C + head + n, DH, stride=PITCH), :] = v[n * DH:(n + 1) * DH]

    def load_head_minor(src, slot, tile, c):
        j = tile * T + c * C
        return src.ref[slot, pl.ds(C + j // H * PITCH + j % H, C), :]

    def transposes(src, dst, cost, store):
        def run(k, j):
            store(k, j, src.load(0, k, 0, T, col=j).T)
        return [Task(cost, [src], [dst], TRANSPOSE_SLACK, run, k, j) for k in range(4) for j in range(4)]

    def wk_sums():
        return sums(RHS, wk_t.load, lambda r, c, v: wk_ops.store(0, r, c, v), [wk_t], [wk_ops], (32, 38))

    def wq_sums():
        return sums(RHS, lambda k, j, c: load_head_minor(wq_t, k, j, c),
                    lambda r, c, v: wq_ops.store(0, r, c, v), [wq_t], [wq_ops], from_f32)

    def pk_sums(r1):
        return interleave(*[
            sums(LHS, lambda j, i, c, b=b: pk.load(b, j * 4 + i, c),
                 lambda r, c, v, b=b: pk_ops.store(b, r, c, v), [pk], [pk_ops], from_f32, [r1])
            for b in range(NB)])

    def z_columns():
        def run(j, c):
            p = [(pk.load(b, j * 4, c) + pk.load(b, j * 4 + 1, c))
                 + (pk.load(b, j * 4 + 2, c) + pk.load(b, j * 4 + 3, c)) for b in range(NB)]
            z = jnp.sum((p[0] + p[1]) + (p[2] + p[3]), axis=1, keepdims=True)
            store_head_minor(wk_t, 0, j * NC + c, jnp.broadcast_to(z, (C, T)))
        return [Task(35, [pk], [wk_t], SUM_SLACK, run, j, c) for j in range(4) for c in range(NC)]

    def z_rows():
        def run(j):
            rows.store(1, 0, j, cat([load_head_minor(wk_t, 0, j, c) for c in range(NC)], 0).T[0:C])
        return [Task(30, [wk_t], [rows], SUM_SLACK, run, j) for j in range(4)]

    def w2_sums(s):
        store = lambda r, c, v: w2_ops.store(0, s * 49 + r, c, v)
        if s == 3:
            return sums(RHS, lambda k, n, c: load_head_minor(w2, n, k, c), store, [w2], [w2_ops], from_f32)
        return sums(RHS, lambda k, n, c: wd.load(0, 4 * s + k, c, col=n), store, [wd], [w2_ops], from_bf16)

    def w2_last_sums():
        def run(n2, c):
            v = {(k, n1): wd.load(0, 12 + k, c, col=2 * n1 + n2) for k, n1 in QUAD}
            for r1 in range(7):
                w2_ops.store(0, 196 + r1 * 2 + n2, c, combine(RHS[r1], lambda i, j: v[i, j]))
        return [Task(25, [wd], [w2_ops], SLACK, run, n2, c) for n2 in range(2) for c in range(NC)]

    def h_sums(b, r1):
        tasks = []
        for s in range(4):
            src, slot, n, first, weight = (pq, 0, 5, 0, pq_weight) if s == 3 else (h, b, 13, 4 * s, h_weight)

            def block(i, k, c, src=src, slot=slot, n=n, first=first, weight=weight):
                return src.load(slot, i * n + first + k, c) * weight.load(0, i, c)
            tasks += sums(LHS, block, lambda r, c, v, s=s: h_ops.store(0, s * 49 + r, c, v),
                          [src], [h_ops], from_bf16, [r1])
        return tasks

    def h_last_sums():
        def run(i2, c):
            v = {(i1, k): h_last.load(0, (2 * i1 + i2) * 2 + k, c) * h_weight.load(0, 2 * i1 + i2, c) for i1, k in QUAD}
            for r1 in range(7):
                h_ops.store(0, 196 + r1 * 2 + i2, c, combine(LHS[r1], lambda i, j: v[i, j]))
        return [Task(25, [h_last], [h_ops], SLACK, run, i2, c) for c in range(NC) for i2 in range(2)]

    def ffn_weights(b):
        def run(i, c):
            p = [x.load(b, i, c, col=j) * rows.load(0, 0, j) for j in range(4)]
            t = jnp.sum((p[0] + p[1]) + (p[2] + p[3]), axis=1, keepdims=True)
            h_weight.store(0, i, c, jnp.broadcast_to(0.5 - 0.5 * jnp.tanh(t), (C, T)))
        return [Task(30, [x], [h_weight], SUM_SLACK, run, i, c) for c in range(NC) for i in range(4)]

    def attention_weights():
        def run(i, c):
            t = den.load(0, i * 2, c) + den.load(0, i * 2 + 1, c)
            t = t + pltpu.roll(t, 2 * H, 1)
            t = t + pltpu.roll(t, H, 1)
            pq_weight.store(0, i, c, (1.0 - h_weight.load(0, i, c)) / (t + 1e-6))
        return [Task(30, [den], [pq_weight], SUM_SLACK + 128, run, i, c) for c in range(NC) for i in range(4)]

    def strassen(fn, lhs, rhs, n, order, finish, writes, extra=None, before=None):
        if stream.aligning and not extra:
            stream.align(n // 4)
        for c in range(0, NC, n // C):
            acc, seen = {}, dict.fromkeys(QUAD, 0)
            for a, r1 in enumerate(order):
                if before:
                    before(a)
                inner = quadrants({r2: stream.product(fn, lhs(r1 * 7 + r2, c, n), rhs(r1 * 7 + r2))
                                   for r2 in (OUT_INNER_ORDER if extra else ORDER)})
                if extra:
                    inner = {q: inner[q] + extra(r1, *q) for q in QUAD}
                for i1, j1, sign in OUT[r1]:
                    for q in QUAD:
                        new = (sign, inner[q])
                        acc[i1, j1, q] = signed_sum([acc[i1, j1, q], new]) if seen[i1, j1] else new
                    seen[i1, j1] += 1
                    if seen[i1, j1] == (4 if i1 == j1 else 2):
                        finish(i1, j1, c, {q: acc[i1, j1, q][1] for q in QUAD})
                        stream.expect(writes, POST_SLACK)

    def ffn_plain(quarters, cols):
        for j in cols:
            for i in quarters:
                def gemm(col):
                    w = pltpu.bitcast(x.ref[0, pl.ds(C + i * T, T), :], u32)
                    return stream.product(dot, [w[:, lanes(k)] for k in range(4)],
                                          w1_first.ref[0, pl.ds(C, D), lanes(col)])
                h.store(0, i * 13 + j, 0, swiglu(gemm(j), gemm(2 + j)))
                stream.expect([h], POST_SLACK)

    def ffn(b, g, n=64, order=ORDER):
        def finish(i1, j1, c, v):
            for i2 in range(2):
                i, act = 2 * i1 + i2, swiglu(v[i2, 0], v[i2, 1])
                if g == NG - 1:
                    h_last.store(0, i * 2 + j1, c, act)
                else:
                    h.store(b, i * 13 + 2 * g + j1, c, act)
        strassen(dot, lambda r, c, n: [x_ops.words(b, r, c, n)],
                 lambda r: w1_ops.operand(g, r), n, order, finish, [h_last if g == NG - 1 else h])

    def keys(b):
        def finish(i1, j1, c, v):
            for i2, j2 in QUAD:
                pk.store(b, (2 * j1 + j2) * 4 + 2 * i1 + i2, c, phi(v[i2, j2]))
        strassen(dot_nt, lambda r, c, n: [wk_ops.words(0, r, c, n)], lambda r: x_ops.operand(b, r),
                 64, ORDER, finish, [pk])

    def queries(b):
        def finish(i1, j1, c, v):
            z = [cat([rows.load(1, 0, 2 * j1 + j2)] * 4, 0) for j2 in range(2)]
            for i2 in range(2):
                i, p = 2 * i1 + i2, [phi(v[i2, j2]) for j2 in range(2)]
                for j2 in range(2):
                    pq.store(0, i * 5 + 2 * j1 + j2, c, p[j2])
                den.store(0, i * 2 + j1, c, p[0] * z[0] + p[1] * z[1])
        strassen(dot_nt, lambda r, c, n: [x_ops.words(b, r, c, n)], lambda r: wq_ops.operand(0, r),
                 64, ORDER, finish, [pq, den])

    def store_quadrant(dst, slot, i1, j1, c, v):
        for i2, j2 in QUAD:
            dst.store(slot, 2 * i1 + i2, c, v[i2, j2], col=2 * j1 + j2)

    def out_copy(b, i1, j1):
        return pltpu.make_async_copy(
            out.ref.at[b, pl.ds(C + i1 * 2 * T, 2 * T), pl.ds(j1 * 2 * T, 2 * T)],
            out_hbm.at[pl.ds(pl.multiple_of((b * 4 + i1 * 2) * T, T), 2 * T), pl.ds(j1 * 2 * T, 2 * T)],
            out_sems.at[b * 4 + i1 * 2 + j1])

    def ungated(tasks):
        return [Task(t.cost, [], t.writes, t.slack, t.run) for t in tasks]

    def run_now(tasks):
        for task in tasks:
            task.run()

    x0 = x_sums(0, (2, 4))
    early = (w1_sums(0, (1,)) + w1_sums(0, (3,)) + x0[:8]
             + w1_sums(0, (6, 0, 4, 2, 5)) + x0[8:] + x_sums(0, (1, 3, 6, 0, 5)))
    wait('x0a', ('w0a', 0), ('w0a', 1))
    stream.host(ungated(early[:6]), 96)
    ffn_plain((0,), (0,))
    wait('x0b')
    stream.host(ungated(early[6:24]), 320)
    ffn_plain((1, 2), (0,))
    wait('x0c', ('w0b', 0), ('w0b', 1))
    stream.host(ungated(early[24:80]), 1088)
    ffn_plain((3,), (0,))
    ffn_plain(range(4), (1,))
    wait('x1')
    tasks = x_sums(1)
    run_now(tasks[:14])
    stream.host(tasks[14:], UNIT * 5 // 8)
    stream.host(early[80:94], UNIT - T, UNIT * 5 // 8)
    ffn(1, 0, 32)
    wait('x2', 'x3')
    tasks = x_sums(2)
    run_now(tasks[:14])
    stream.host(tasks[14:], UNIT * 5 // 8)
    stream.host(x_sums(3) + early[94:], 2 * UNIT - T, UNIT * 5 // 8)
    ffn(2, 0, 32)
    ffn(3, 0, 32)

    wait((1, 0), (1, 1), 'gw', 'wk', (2, 0), (2, 1))
    tasks = sum([w1_sums(1, [r1]) for r1 in COLD_ORDER], [])
    run_now(tasks[:17])
    stream.host(tasks[17:], 1050)
    tasks = w1_sums(2)
    stream.host(transposes(wk, wk_t, 70, lambda k, j, v: wk_t.store(k, j, 0, v)) + tasks[:14] + wk_sums(),
                4 * UNIT - SLACK, UNIT - SLACK)
    ffn(0, 1, T, COLD_ORDER)
    for b in range(1, NB):
        ffn(b, 1)
    stream.host(tasks[14:], 4 * UNIT - POST_SLACK)
    for b in range(NB):
        keys(b)
    half_gw = 0.5 * gw_ref[...].astype(f32).reshape(1, D)
    for j in range(4):
        rows.store(0, 0, j, jnp.broadcast_to(half_gw[:, lanes(j)], (C, T)))

    wait(*[(g, u) for g in range(3, NG) for u in range(2)], 'wq', 'wv', 'wo', 'wd')
    stream.aligning = True
    tasks = w1_sums(3) + w1_sums(4) + w1_sums(5) + w1_sums(6)
    stream.host(tasks[:35] + pk_sums(WIDE_ORDER[0]) + pk_sums(WIDE_ORDER[1]), 2 * UNIT)
    ffn(0, 2)
    ffn(1, 2)
    stream.host(interleave(sum([pk_sums(r1) for r1 in WIDE_ORDER[2:]], []) + z_columns(),
                           tasks[35:147] + ffn_weights(0) + w2_last_sums()), 4 * UNIT)
    strassen(dot, lambda r, c, n: [pk_ops.words(b, r, c, n) for b in range(NB)],
             lambda r: cat([x_ops.operand(b, L2R[r // 7] * 7 + L2R[r % 7]) for b in range(NB)], 0),
             T, WIDE_ORDER, lambda *a: store_quadrant(pkx, 0, *a), [pkx])
    stream.host(transposes(wq, wq_t, 60, lambda k, j, v: store_head_minor(wq_t, k, j * NC, v)) + z_rows()
                + wq_sums() + tasks[147:] + sum([w2_sums(s) for s in range(4)], []), 10 * UNIT - 224, 64)
    ffn(2, 2)
    same_head = (lax.broadcasted_iota(jnp.int32, (T, T), 0) // DH
                 == lax.broadcasted_iota(jnp.int32, (T, T), 1) // DH)
    kv = [jnp.where(same_head, dot(pkx.ref[0, pl.ds(C + j * T, T), :], wv_ref[:, lanes(j)]), 0.0).astype(bf16)
          for j in range(4)]
    ffn(3, 2)
    for j in range(4):
        v = dot(kv[j], wo_ref[lanes(j), :])
        for n in range(4):
            store_head_minor(w2, n, j * NC, v[:, lanes(n)])
    stream.recent = []
    stream.expect([w2], SLACK)
    for g in (3, 4):
        for b in range(NB):
            ffn(b, g)

    @pl.loop(0, NB)
    def _(b):
        stream.restart()
        queries(b)
        stream.host(attention_weights() + h_sums(b, WIDE_ORDER[0]), 2 * UNIT - 288)
        ffn(b, 5)
        ffn(b, 6)

        def before(a):
            if a < 6:
                stream.host((h_last_sums() if a == 0 else []) + h_sums(b, WIDE_ORDER[a + 1]), 8 * T - 192)
            else:
                stream.host(ffn_weights((b + 1) % NB), 8 * T - SUM_SLACK)

        def finish(i1, j1, c, v):
            store_quadrant(out, b, i1, j1, c, v)
            out_copy(b, i1, j1).start()

        strassen(dot, lambda r, c, n: [h_ops.words(0, s * 49 + r, c, n) for s in range(4)],
                 lambda r: cat([w2_ops.operand(0, s * 49 + r) for s in range(4)], 0),
                 T, WIDE_ORDER, finish, [out], before=before,
                 extra=lambda r1, i2, j2: stream.product(dot, [h_ops.words(0, 196 + r1 * 2 + i2)],
                                                         w2_ops.operand(0, 196 + r1 * 2 + j2)))
        stream.restart()

    for b in range(NB):
        for q in QUAD:
            out_copy(b, *q).wait()


@jax.jit
def pallas_gated_mix__linear_attn_block__swiglu_ffn__prompt_kernel(
    A_x: jax.Array,
    A_wqkv: jax.Array,
    A_wo: jax.Array,
    B_x: jax.Array,
    B_w_gate: jax.Array,
    B_w_up: jax.Array,
    B_w_down: jax.Array,
    gate_w: jax.Array,
):
    del B_x

    def scratch(slots, tiles, width, dtype):
        n = C + tiles * tile_pitch(width, dtype)
        return pltpu.VMEM((slots, -(-n // 64) * 64, width), dtype)

    hbm = pl.BlockSpec(memory_space=pl.ANY)
    result = pl.pallas_call(
        kernel,
        in_specs=[hbm] * 7,
        out_specs=hbm,
        out_shape=jax.ShapeDtypeStruct((S, D), bf16),
        scratch_shapes=[
            pltpu.VMEM((D, D), bf16), pltpu.VMEM((D, D), bf16), pltpu.VMEM((D,), bf16),
            pltpu.SMEM((2,), jnp.int32), pltpu.SemaphoreType.DMA((28,)), pltpu.SemaphoreType.DMA((4 * NB,)),
            *[scratch(*spec) for spec in BUFFERS.values()]],
        compiler_params=pltpu.CompilerParams(
            vmem_limit_bytes=112 * 1024 * 1024, disable_bounds_checks=True, disable_semaphore_checks=True),
    )(A_x.reshape(S, D), A_wqkv, A_wo, B_w_gate, B_w_up, B_w_down, gate_w)
    return result.reshape(1, S, D)
```
